```python
import jax
import jax.numpy as jnp

def _softmax(x, axis=-1):
    return jax.nn.softmax(x, axis=axis)

def _gelu(x):
    return jax.nn.gelu(x, approximate=True)

def _silu(x):
    return jax.nn.silu(x)

def _sigmoid(x):
    return jax.nn.sigmoid(x)

def _layernorm(x, axis=-1, eps=1e-05):
    m = jnp.mean(x, axis=axis, keepdims=True)
    v = jnp.var(x, axis=axis, keepdims=True)
    return (x - m) / jnp.sqrt(v + eps)

def _scatter_add(tgt, idx, src, axis=0):
    return tgt.at[idx].add(src)

def _segment_sum(src, seg, n):
    return jax.ops.segment_sum(src, seg, n)

class _Rng:

    def __init__(self, key):
        self._k = key

    def _next(self):
        self._k, sub = jax.random.split(self._k)
        return sub

    def normal(self, shape):
        return jax.random.normal(self._next(), shape, dtype=jnp.bfloat16)

    def randint(self, lo, hi, shape):
        return jax.random.randint(self._next(), shape, lo, hi, dtype=jnp.int32)

    def uniform(self, shape, lo=0.0, hi=1.0):
        return jax.random.uniform(self._next(), shape, jnp.bfloat16, lo, hi)

    def permutation(self, n):
        return jax.random.permutation(self._next(), n)
kernel_name = 'adaLN_cond__sliding_block_cached__mixer_channel_mlp__decode'

def setup_inputs():
    _rng = _Rng(jax.random.key(int.from_bytes(__import__("os").urandom(4), "little")))
    _w = lambda a: (lambda t: t.astype(jnp.bfloat16) if jnp.issubdtype(t.dtype, jnp.floating) else t)(jnp.asarray(a))

    def _A_setup():
        B, Sq, D = (8, 1, 640)
        Hq, Hkv, Sk, Dh = (32, 32, 4096, 192)
        assert Hq % Hkv == 0, (Hq, Hkv)
        return {'x': _w((lambda *s: _rng.normal(s) * 0.05)(B, Sq, D)), 'k_cache': _w((lambda *s: _rng.normal(s) * 0.05)(B, Hkv, Sk, Dh)), 'v_cache': _w((lambda *s: _rng.normal(s) * 0.05)(B, Hkv, Sk, Dh)), 'wq': _w((lambda *s: _rng.normal(s) * 0.05)(D, Hq * Dh) * D ** (-0.5)), 'wo': _w((lambda *s: _rng.normal(s) * 0.05)(Hq * Dh, D) * (Hq * Dh) ** (-0.5))}
    _A_in = _A_setup()

    def _B_setup():
        B, S, D, F = (8, 1, 640, 1536)
        return {'x': _w((lambda *s: _rng.normal(s) * 0.05)(B, S, D)), 'w1': _w((lambda *s: _rng.normal(s) * 0.05)(D, F) * D ** (-0.5)), 'b1': _w((lambda *s: _rng.normal(s) * 0.05)(F)), 'w2': _w((lambda *s: _rng.normal(s) * 0.05)(F, D) * F ** (-0.5)), 'b2': _w((lambda *s: _rng.normal(s) * 0.05)(D))}
    _B_in = _B_setup()
    return {'A_x': _A_in['x'], 'A_k_cache': _A_in['k_cache'], 'A_v_cache': _A_in['v_cache'], 'A_wq': _A_in['wq'], 'A_wo': _A_in['wo'], 'B_x': _B_in['x'], 'B_w1': _B_in['w1'], 'B_b1': _B_in['b1'], 'B_w2': _B_in['w2'], 'B_b2': _B_in['b2'], 'c': _w((lambda *s: _rng.normal(s) * 0.05)(8, 640)), 'w_mod': _w((lambda *s: _rng.normal(s) * 0.05)(640, 6 * 640) * 640 ** (-0.5))}

def reference(A_x, A_k_cache, A_v_cache, A_wq, A_wo, B_x, B_w1, B_b1, B_w2, B_b2, c, w_mod):

    def _A_ref(x, k_cache, v_cache, wq, wo):
        B, Sq, D = x.shape
        Hq, Dh = (32, 192)
        Hkv, Sk = (k_cache.shape[1], k_cache.shape[2])
        W = min(4096, max(256, Sk // 4))
        rep = Hq // Hkv
        q = (lambda x, *d: x.transpose(*d))((x @ wq).reshape(B, Sq, Hq, Dh), 0, 2, 1, 3)
        k = jnp.repeat(k_cache[:, :, Sk - W:, :], rep, axis=1)
        v = jnp.repeat(v_cache[:, :, Sk - W:, :], rep, axis=1)
        scores = jnp.einsum('bhqd,bhkd->bhqk', q, k) * Dh ** (-0.5)
        p = _softmax(scores, axis=-1)
        o = jnp.einsum('bhqk,bhkd->bhqd', p, v)
        return (lambda x, *d: x.transpose(*d))(o, 0, 2, 1, 3).reshape(B, Sq, Hq * Dh) @ wo

    def _B_ref(x, w1, b1, w2, b2):
        y = _layernorm(x, axis=-1)
        h = _gelu(jnp.einsum('bsd,df->bsf', y, w1) + b1)
        return jnp.einsum('bsf,fd->bsd', h, w2) + b2
    x = A_x
    mod = (_silu(c) @ w_mod).reshape(c.shape[0], 6, 1, -1)
    sa, ca, ga, sb, cb, gb = (mod[:, 0].copy(), mod[:, 1].copy(), mod[:, 2].copy(), mod[:, 3].copy(), mod[:, 4].copy(), mod[:, 5].copy())
    h = _layernorm(x, axis=-1) * (1 + ca) + sa
    x = x + ga * _A_ref(h, A_k_cache, A_v_cache, A_wq, A_wo)
    h = _layernorm(x, axis=-1) * (1 + cb) + sb
    x = x + gb * _B_ref(h, B_w1, B_b1, B_w2, B_b2)
    return x
```

```python
import functools
import itertools

import jax
import jax.numpy as jnp
from jax import lax
import jax.experimental.pallas as pl
import jax.experimental.pallas.tpu as pltpu

B, D, H, SK, DH, F = 8, 640, 32, 4096, 192, 1536
W = min(4096, max(256, SK // 4))
NP = H // 2
PW = 2 * DH
EPS = 1e-5
NSLOT = 3


def _ln(x):
    m = jnp.mean(x, axis=-1, keepdims=True)
    xc = x - m
    v = jnp.mean(xc * xc, axis=-1, keepdims=True)
    return xc / jnp.sqrt(v + EPS)


def _dot(a, b):
    return jnp.dot(a, b, preferred_element_type=jnp.float32)


def _dot_nt(a, b):
    return lax.dot_general(a, b, (((1,), (1,)), ((), ())), preferred_element_type=jnp.float32)


def _kernel(x_ref, c_ref, b1_ref, b2_ref,
            k_hbm, v_hbm, wq_hbm, wo_hbm, w1_hbm, w2_hbm, wm_hbm,
            o_ref,
            kbuf, vbuf, wq_v, wo_v, w1_v, w2_v, wm_v, q_v, kv_sem, w_sem):
    col0 = SK - W

    def kv_dmas(j, slot, part):
        n = 0
        for r in range(part * 6, part * 6 + 6):
            for src, dst in ((k_hbm, kbuf), (v_hbm, vbuf)):
                for jc in range(2):
                    for jb in range(2):
                        pltpu.make_async_copy(
                            src.at[pl.ds(jb * 4, 4), j, pl.ds(r * 8, 8), pl.ds(col0 + jc * 512, 512)],
                            dst.at[slot, pl.ds(jb * 4, 4), pl.ds(r * 8, 8), pl.ds(jc * 512, 512)],
                            kv_sem.at[slot]).start(priority=n % 2)
                        n += 1

    def kv_wait(slot):
        pltpu.make_async_copy(kbuf.at[slot], kbuf.at[slot], kv_sem.at[slot]).wait()
        pltpu.make_async_copy(vbuf.at[slot], vbuf.at[slot], kv_sem.at[slot]).wait()

    cp_wm = pltpu.make_async_copy(wm_hbm, wm_v, w_sem.at[0])
    cp_wq = pltpu.make_async_copy(wq_hbm, wq_v, w_sem.at[1])
    cp_wo = pltpu.make_async_copy(wo_hbm, wo_v, w_sem.at[2])
    cp_w1 = pltpu.make_async_copy(w1_hbm, w1_v, w_sem.at[3])
    cp_w2 = pltpu.make_async_copy(w2_hbm, w2_v, w_sem.at[4])
    cp_wm.start()
    cp_wq.start(priority=1)
    cp_wo.start()
    cp_w1.start(priority=1)
    cp_w2.start()
    for j in range(NSLOT - 1):
        for part in range(8):
            kv_dmas(j, j, part)

    x = x_ref[...].astype(jnp.float32)
    cc = c_ref[...].astype(jnp.float32)
    sc = (cc * jax.nn.sigmoid(cc)).astype(jnp.bfloat16)
    cp_wm.wait()
    mod = _dot(sc, wm_v[...])
    sa, ca, ga, sb, cb, gb = (mod[:, i * D:(i + 1) * D] for i in range(6))
    h = _ln(x) * (1.0 + ca) + sa
    cp_wq.wait()
    q_v[...] = _dot(h.astype(jnp.bfloat16), wq_v[...])
    cp_wo.wait()

    row16 = lax.broadcasted_iota(jnp.int32, (16, PW), 0)
    lane16 = lax.broadcasted_iota(jnp.int32, (16, PW), 1)
    diag = (row16 < 8) == (lane16 < DH)
    rowb_s = lax.broadcasted_iota(jnp.int32, (16, W), 0) % 8
    rowb_o = row16 % 8
    lane8 = lax.broadcasted_iota(jnp.int32, (8, PW), 1)
    scale = DH ** -0.5

    def pair(j, acc):
        slot = j % NSLOT
        nslot = (j + NSLOT - 1) % NSLOT
        off = pl.multiple_of(j * PW, 128)
        q2 = q_v[:, pl.ds(off, PW)]
        q16 = jnp.where(diag, jnp.concatenate([q2, q2], axis=0), 0.0).astype(jnp.bfloat16)
        kv_wait(slot)
        s = jnp.zeros((16, W), jnp.float32)
        for b in range(B):
            if b % 2 == 0:
                @pl.when(j + NSLOT - 1 < NP)
                def _():
                    kv_dmas(j + NSLOT - 1, nslot, b // 2)
            s = jnp.where(rowb_s == b, _dot(q16, kbuf[slot, b]), s)
        s = s * scale
        m = jnp.max(s, axis=-1, keepdims=True)
        e = jnp.exp(s - m)
        p = (e / jnp.sum(e, axis=-1, keepdims=True)).astype(jnp.bfloat16)
        o = jnp.zeros((16, PW), jnp.float32)
        for b in range(B):
            if b % 2 == 0:
                @pl.when(j + NSLOT - 1 < NP)
                def _():
                    kv_dmas(j + NSLOT - 1, nslot, 4 + b // 2)
            o = jnp.where(rowb_o == b, _dot_nt(p, vbuf[slot, b]), o)
        o2 = jnp.where(lane8 < DH, o[:8], o[8:]).astype(jnp.bfloat16)
        return acc + _dot(o2, wo_v[pl.ds(off, PW), :])

    attn = lax.fori_loop(0, NP, pair, jnp.zeros((B, D), jnp.float32))
    x1 = x + ga * attn
    h2 = _ln(x1) * (1.0 + cb) + sb
    y = _ln(h2)
    cp_w1.wait()
    u = _dot(y.astype(jnp.bfloat16), w1_v[...]) + b1_ref[...].astype(jnp.float32).reshape(1, F)
    g = jax.nn.gelu(u, approximate=True)
    cp_w2.wait()
    mlp = _dot(g.astype(jnp.bfloat16), w2_v[...]) + b2_ref[...].astype(jnp.float32).reshape(1, D)
    o_ref[...] = (x1 + gb * mlp).astype(o_ref.dtype)


@jax.jit
def pallas_adaLN_cond__sliding_block_cached__mixer_channel_mlp__decode_kernel(
    A_x, A_k_cache, A_v_cache, A_wq, A_wo, B_x, B_w1, B_b1, B_w2, B_b2, c, w_mod,
):
    del B_x
    kt = jnp.swapaxes(A_k_cache, 2, 3).reshape(B, NP, PW, SK)
    vt = jnp.swapaxes(A_v_cache, 2, 3).reshape(B, NP, PW, SK)
    vmem = pl.BlockSpec(memory_space=pltpu.VMEM)
    hbm = pl.BlockSpec(memory_space=pl.ANY)
    bf = jnp.bfloat16
    out = pl.pallas_call(
        _kernel,
        in_specs=[vmem] * 4 + [hbm] * 7,
        out_specs=vmem,
        out_shape=jax.ShapeDtypeStruct((B, D), A_x.dtype),
        scratch_shapes=[
            pltpu.VMEM((NSLOT, B, PW, W), bf),
            pltpu.VMEM((NSLOT, B, PW, W), bf),
            pltpu.VMEM((D, H * DH), bf),
            pltpu.VMEM((H * DH, D), bf),
            pltpu.VMEM((D, F), bf),
            pltpu.VMEM((F, D), bf),
            pltpu.VMEM((D, 6 * D), bf),
            pltpu.VMEM((B, H * DH), jnp.float32),
            pltpu.SemaphoreType.DMA((NSLOT,)),
            pltpu.SemaphoreType.DMA((5,)),
        ],
        compiler_params=pltpu.CompilerParams(
            vmem_limit_bytes=100 * 2**20, disable_bounds_checks=True),
    )(A_x.reshape(B, D), c, B_b1, B_b2, kt, vt, A_wq, A_wo, B_w1, B_w2, w_mod)
    return out.reshape(B, 1, D)
```

```python
import functools
import itertools

import jax
import jax.numpy as jnp
from jax import lax
import jax.experimental.pallas as pl
import jax.experimental.pallas.tpu as pltpu

B, D, H, SK, DH, F = 8, 640, 32, 4096, 192, 1536
W = min(4096, max(256, SK // 4))
NP = H // 2
PW = 2 * DH
EPS = 1e-5

CFG = dict(nb=2, nc=1024, order='dcbh', unroll_b=False, compute=True,
           wq='a', wo_rows=32, wa='x', wt='x', skip=(), mix=False, w2_rows=24)


def _ln(x):
    m = jnp.mean(x, axis=-1, keepdims=True)
    xc = x - m
    v = jnp.mean(xc * xc, axis=-1, keepdims=True)
    return xc / jnp.sqrt(v + EPS)


def _dot(a, b):
    return jnp.dot(a, b, preferred_element_type=jnp.float32)


def _dot_nt(a, b):
    return lax.dot_general(a, b, (((1,), (1,)), ((), ())), preferred_element_type=jnp.float32)


def _ds(start, size, mult):
    if isinstance(start, int):
        return pl.ds(start, size)
    return pl.ds(pl.multiple_of(start, mult), size)


def _kernel(cfg, x_hbm, c_hbm, b1_hbm, b2_hbm,
            k_hbm, v_hbm, wq_hbm, wo_hbm, w1_hbm, w2_hbm, wm_hbm,
            o_ref,
            kbuf, vbuf, wq_v, wo_v, w1_v, w2_v, wma_v, wmb_v, wmc_v, q_v,
            x_v, c_v, b1_v, b2_v, k_sem, v_sem, w_sem):
    col0 = SK - W
    nb, nc, order = cfg['nb'], cfg['nc'], cfg['order']
    skip = cfg['skip']

    def start_all(lst):
        for n, (src, dst, sem) in enumerate(lst):
            pltpu.make_async_copy(src, dst, sem).start(priority=n % 2)

    def cache_part(src, dst, sem, j, slot, part):
        rng = dict(d=3, c=W // nc, b=B // nb, h=2)
        lst = []
        for idx in itertools.product(*[range(rng[o]) for o in order]):
            i = dict(zip(order, idx))
            r = _ds(i['h'] * DH + (part * 3 + i['d']) * 8, 8, 8)
            bs = pl.ds(i['b'] * nb, nb)
            lst.append((src.at[bs, j, r, pl.ds(col0 + i['c'] * nc, nc)],
                        dst.at[slot, bs, r, pl.ds(i['c'] * nc, nc)], sem.at[slot]))
        start_all(lst)

    def wq_part(part):
        if 'wq' in skip: return
        lst = []
        if cfg['wq'] == 'a':
            idx = [(i * 8 + part, c) for c in range(6) for i in range(5)]
        elif cfg['wq'] == 'b':
            idx = [(i * 8 + part, (c + i) % 6) for c in range(6) for i in range(5)]
        elif cfg['wq'] == 'c':
            idx = [(i * 8 + part, c) for i in range(5) for c in range(6)]
        elif cfg['wq'] == 'd':
            idx = [(part * 5 + i, c) for i in range(5) for c in range(6)]
        elif cfg['wq'] == 'e':
            idx = [(i * 4 + part % 4, c * 2 + part // 4) for c in range(3) for i in range(10)]
        for r, c in idx:
            rs = _ds(r * 8, 8, 8); cs = _ds(c * 1024, 1024, 128)
            lst.append((wq_hbm.at[:, rs, cs], wq_v.at[:, rs, cs], w_sem.at[9]))
        start_all(lst)

    def wo_part(part):
        if 'wo' in skip: return
        n = cfg['wo_rows']
        per = H * DH // n // 8
        lst = []
        for i in range(per):
            r = _ds((i * 8 + part) * n, n, 8)
            lst.append((wo_hbm.at[r, :], wo_v.at[r, :], w_sem.at[10]))
        start_all(lst)

    def rows(part, i, n, size, mode):
        if mode == 'seq':
            return _ds((part * n + i) * size, size, 8)
        return _ds((i * 8 + part) * size, size, 8)

    def tail_a(part):
        if 'wt' in skip: return
        l0 = []; l1 = []
        for i in range(10):
            r = rows(part, i, 10, 8, cfg['wt'])
            l0.append((wm_hbm.at[r, pl.ds(2 * D, 3 * D)], wmb_v.at[r, :], w_sem.at[1]))
            l1.append((w1_hbm.at[r, :], w1_v.at[r, :], w_sem.at[2]))
        if cfg.get('mix'):
            start_all([x for p in zip(l0, l1) for x in p])
        else:
            start_all(l0 + l1)

    def tail_b(part):
        if 'wt' in skip: return
        lst = []
        n = cfg['w2_rows']; per = F // n // 8
        for i in range(per):
            r = rows(part, i, per, n, cfg['wt'])
            lst.append((w2_hbm.at[r, :], w2_v.at[r, :], w_sem.at[3]))
        start_all(lst)

    def tail_c():
        if 'wt' in skip: return
        lst = []
        for part in range(8):
            for i in range(5):
                r = rows(part, i, 5, 16, cfg['wt'])
                lst.append((wm_hbm.at[r, pl.ds(5 * D, D)], wmc_v.at[r, :], w_sem.at[4]))
        start_all(lst)

    def wait_all(buf, sem):
        pltpu.make_async_copy(buf, buf, sem).wait()

    def loop8(body, init):
        if cfg['unroll_b']:
            for b in range(8):
                init = body(b, init)
            return init
        return lax.fori_loop(0, 8, body, init)

    def first(part, _):
        lst = []
        for i in range(10):
            r = rows(part, i, 10, 8, cfg['wa'])
            lst.append((wm_hbm.at[r, pl.ds(0, 2 * D)], wma_v.at[r, :], w_sem.at[0]))
        start_all(lst)
        return _
    if 'wa' not in skip: lax.fori_loop(0, 8, first, 0)
    small = [pltpu.make_async_copy(s, d, w_sem.at[5 + i]) for i, (s, d) in enumerate(
        ((x_hbm, x_v), (c_hbm, c_v), (b1_hbm, b1_v), (b2_hbm, b2_v)))]
    for cp in small:
        cp.start()
    lax.fori_loop(0, 8, lambda part, _: wq_part(part), None)

    for cp in small:
        cp.wait()
    x = x_v[...].astype(jnp.float32)
    cc = c_v[...].astype(jnp.float32)
    sc = (cc * jax.nn.sigmoid(cc)).astype(jnp.bfloat16)
    if 'wa' not in skip: wait_all(wma_v, w_sem.at[0])
    mod_a = _dot(sc, wma_v[...])
    h = (_ln(x) * (1.0 + mod_a[:, D:]) + mod_a[:, :D]).astype(jnp.bfloat16)

    lax.fori_loop(0, 8, lambda part, _: cache_part(k_hbm, kbuf, k_sem, 0, 0, part), None)
    if 'wq' not in skip: wait_all(wq_v, w_sem.at[9])

    def q_part(part, _):
        wo_part(part)
        cs = _ds(part * 2 * PW, 2 * PW, 128)
        q_v[:, cs] = _dot(h, wq_v[:, :, cs].reshape(D, 2 * PW))
        return _
    lax.fori_loop(0, 8, q_part, 0)
    lax.fori_loop(0, 8, lambda part, _: cache_part(v_hbm, vbuf, v_sem, 0, 0, part), None)
    if 'wo' not in skip: wait_all(wo_v, w_sem.at[10])

    row16 = lax.broadcasted_iota(jnp.int32, (16, PW), 0)
    lane16 = lax.broadcasted_iota(jnp.int32, (16, PW), 1)
    diag = (row16 < 8) == (lane16 < DH)
    row_s = lax.broadcasted_iota(jnp.int32, (16, W), 0) % 8
    row_o = row16 % 8
    lane8 = lax.broadcasted_iota(jnp.int32, (8, PW), 1)
    scale = DH ** -0.5

    def pair(j, acc):
        slot = j % 2
        nslot = 1 - slot
        off = _ds(j * PW, PW, 128)
        q2 = q_v[:, off]
        q16 = jnp.where(diag, jnp.concatenate([q2, q2], axis=0), 0.0).astype(jnp.bfloat16)
        wait_all(kbuf.at[slot], k_sem.at[slot])

        def qk(b, s):
            pl.when(j + 1 < NP)(lambda: cache_part(k_hbm, kbuf, k_sem, j + 1, nslot, b))
            pl.when(j + 1 == NP)(lambda: tail_a(b))
            if not cfg['compute']: return s
            return jnp.where(row_s == b, _dot(q16, kbuf[slot, b]), s)

        s = loop8(qk, jnp.zeros((16, W), jnp.float32)) * scale
        m = jnp.max(s, axis=-1, keepdims=True)
        e = jnp.exp(s - m)
        p = (e / jnp.sum(e, axis=-1, keepdims=True)).astype(jnp.bfloat16)
        wait_all(vbuf.at[slot], v_sem.at[slot])

        def pv(b, o):
            pl.when(j + 1 < NP)(lambda: cache_part(v_hbm, vbuf, v_sem, j + 1, nslot, b))
            pl.when(j + 1 == NP)(lambda: tail_b(b))
            if not cfg['compute']: return o
            return jnp.where(row_o == b, _dot_nt(p, vbuf[slot, b]), o)

        o = loop8(pv, jnp.zeros((16, PW), jnp.float32))
        o2 = jnp.where(lane8 < DH, o[:8], o[8:]).astype(jnp.bfloat16)
        return acc + _dot(o2, wo_v[off, :])

    attn = lax.fori_loop(0, NP, pair, jnp.zeros((B, D), jnp.float32))
    tail_c()
    if 'wt' not in skip: wait_all(wmb_v, w_sem.at[1])
    mod_b = _dot(sc, wmb_v[...])
    ga, sb, cb = (mod_b[:, i * D:(i + 1) * D] for i in range(3))
    x1 = x + ga * attn
    h2 = _ln(x1) * (1.0 + cb) + sb
    y = _ln(h2)
    if 'wt' not in skip: wait_all(w1_v, w_sem.at[2])
    u = _dot(y.astype(jnp.bfloat16), w1_v[...]) + b1_v[...].astype(jnp.float32).reshape(1, F)
    g = jax.nn.gelu(u, approximate=True)
    if 'wt' not in skip: wait_all(w2_v, w_sem.at[3])
    mlp = _dot(g.astype(jnp.bfloat16), w2_v[...]) + b2_v[...].astype(jnp.float32).reshape(1, D)
    if 'wt' not in skip: wait_all(wmc_v, w_sem.at[4])
    gb = _dot(sc, wmc_v[...])
    o_ref[...] = (x1 + gb * mlp).astype(o_ref.dtype)


def make(**over):
    cfg = dict(CFG, **over)

    @jax.jit
    def fn(A_x, A_k_cache, A_v_cache, A_wq, A_wo, B_x, B_w1, B_b1, B_w2, B_b2, c, w_mod):
        del B_x
        kt = jnp.swapaxes(A_k_cache, 2, 3).reshape(B, NP, PW, SK)
        vt = jnp.swapaxes(A_v_cache, 2, 3).reshape(B, NP, PW, SK)
        hbm = pl.BlockSpec(memory_space=pl.ANY)
        bf = jnp.bfloat16
        out = pl.pallas_call(
            functools.partial(_kernel, cfg),
            in_specs=[hbm] * 11,
            out_specs=pl.BlockSpec(memory_space=pltpu.VMEM),
            out_shape=jax.ShapeDtypeStruct((B, D), A_x.dtype),
            scratch_shapes=[
                pltpu.VMEM((2, B, PW, W), bf),
                pltpu.VMEM((2, B, PW, W), bf),
                pltpu.VMEM((2, D // 2, H * DH), bf),
                pltpu.VMEM((H * DH, D), bf),
                pltpu.VMEM((D, F), bf),
                pltpu.VMEM((F, D), bf),
                pltpu.VMEM((D, 2 * D), bf),
                pltpu.VMEM((D, 3 * D), bf),
                pltpu.VMEM((D, D), bf),
                pltpu.VMEM((B, H * DH), jnp.float32),
                pltpu.VMEM((B, D), bf),
                pltpu.VMEM((B, D), bf),
                pltpu.VMEM((F,), bf),
                pltpu.VMEM((D,), bf),
                pltpu.SemaphoreType.DMA((2,)),
                pltpu.SemaphoreType.DMA((2,)),
                pltpu.SemaphoreType.DMA((11,)),
            ],
            compiler_params=pltpu.CompilerParams(
                vmem_limit_bytes=64 * 2**20, disable_bounds_checks=True),
        )(A_x.reshape(B, D), c, B_b1, B_b2, kt, vt, A_wq.reshape(2, D // 2, H * DH),
          A_wo, B_w1, B_w2, w_mod)
        return out.reshape(B, 1, D)
    return fn


pallas_adaLN_cond__sliding_block_cached__mixer_channel_mlp__decode_kernel = make()
```

```python
import jax
import jax.numpy as jnp
from jax import lax
import jax.experimental.pallas as pl
import jax.experimental.pallas.tpu as pltpu

B, D, H, SK, DH, F = 8, 640, 32, 4096, 192, 1536
W = min(4096, max(256, SK // 4))
NP = H // 2
PW = 2 * DH
EPS = 1e-5
W2_SPLIT = 1024


def _layernorm(x):
    xc = x - jnp.mean(x, axis=-1, keepdims=True)
    return xc / jnp.sqrt(jnp.mean(xc * xc, axis=-1, keepdims=True) + EPS)


def _dot(a, b):
    return jnp.dot(a, b, preferred_element_type=jnp.float32)


def _dot_nt(a, b):
    return lax.dot_general(a, b, (((1,), (1,)), ((), ())), preferred_element_type=jnp.float32)


def _rows(group, size):
    if isinstance(group, int):
        return pl.ds(group * size, size)
    return pl.ds(pl.multiple_of(group * size, 8), size)


def _cols(group, size):
    return pl.ds(pl.multiple_of(group * size, 128), size)


def _start(copies, sem):
    for n, (src, dst) in enumerate(copies):
        pltpu.make_async_copy(src, dst, sem).start(priority=n % 2)


def _wait(buf, sem):
    pltpu.make_async_copy(buf, buf, sem).wait()


def _repeat(n, body):
    lax.fori_loop(0, n, lambda i, _: body(i), None)


def _kernel(x_hbm, c_hbm, b1_hbm, b2_hbm, k_hbm, v_hbm, wq_hbm, wo_hbm, w1_hbm, w2_hbm, wm_hbm,
            o_ref,
            k_buf, v_buf, wq_buf, wo_buf, w1_buf, w2_buf, wm_buf, q_buf, mod_buf,
            x_buf, c_buf, b1_buf, b2_buf, sems):
    sem_k, sem_v, sem_w = sems.at[0], sems.at[1], sems.at[2]

    def fetch_cache(src, dst, sem, pair, part):
        copies = []
        for i in range(3):
            for b in range(0, B, 2):
                for h in range(2):
                    r = _rows(h * (DH // 8) + part * 3 + i, 8)
                    copies.append((src.at[pl.ds(b, 2), pair, r, pl.ds(SK - W, W)],
                                   dst.at[pair % 2, pl.ds(b, 2), r, :]))
        _start(copies, sem)

    def fetch_wm(part):
        copies = []
        for tile, width in ((0, 8), (15, 8), (8, 7), (23, 7)):
            for i in range(8):
                r, c = _rows(i * 5 + part, 8), pl.ds(tile * 128, width * 128)
                copies.append((wm_hbm.at[:, r, c], wm_buf.at[:, r, c]))
        _start(copies, sem_w)

    def fetch_wq(part):
        copies = []
        for col in range(6):
            for i in range(8):
                r, c = _rows(i * 5 + part, 8), pl.ds(col * 1024, 1024)
                copies.append((wq_hbm.at[:, r, c], wq_buf.at[:, r, c]))
        _start(copies, sem_v)

    def fetch_wo(part):
        rows = [_rows(i * 16 + part * 2 + t, 24) for t in range(2) for i in range(16)]
        _start([(wo_hbm.at[r, :], wo_buf.at[r, :]) for r in rows], sem_w)

    def fetch_w1(part):
        rows = [_rows(i * 8 + part, 8) for i in range(10)]
        _start([(w1_hbm.at[r, :], w1_buf.at[r, :]) for r in rows], sem_k)

    def fetch_w2_head(part):
        rows = [_rows(i * 8 + part, 32) for i in range(W2_SPLIT // 256)]
        _start([(w2_hbm.at[r, :], w2_buf.at[r, :]) for r in rows], sem_v)

    def fetch_w2_rest():
        rows = [_rows(W2_SPLIT // 32 + i * 4 + t, 32)
                for t in range(4) for i in range((F - W2_SPLIT) // 128)]
        _start([(w2_hbm.at[r, :], w2_buf.at[r, :]) for r in rows], sem_w)

    _repeat(5, fetch_wm)
    small = [pltpu.make_async_copy(src, dst, sem_k) for src, dst in
             ((x_hbm, x_buf), (c_hbm, c_buf), (b1_hbm, b1_buf), (b2_hbm, b2_buf))]
    for copy in small:
        copy.start()
    _repeat(2, fetch_wq)
    for copy in small:
        copy.wait()
    _wait(wm_buf, sem_w)

    x = x_buf[...].astype(jnp.float32)
    silu_c = jax.nn.silu(c_buf[...].astype(jnp.float32)).astype(jnp.bfloat16)

    def modulation(i):
        pl.when(i < 3)(lambda: fetch_wq(2 + i))
        mod_buf[i] = _dot(silu_c, wm_buf[:, :, _cols(i, D)].reshape(D, D))

    _repeat(6, modulation)
    h = (_layernorm(x) * (1.0 + mod_buf[1]) + mod_buf[0]).astype(jnp.bfloat16)

    _repeat(8, lambda part: fetch_cache(k_hbm, k_buf, sem_k, 0, part))
    _wait(wq_buf, sem_v)

    def queries(i):
        fetch_wo(i)
        c = _cols(i, 2 * PW)
        q_buf[:, c] = _dot(h, wq_buf[:, :, c].reshape(D, 2 * PW))

    _repeat(8, queries)
    _repeat(8, lambda part: fetch_cache(v_hbm, v_buf, sem_v, 0, part))
    _wait(wo_buf, sem_w)

    row = lax.broadcasted_iota(jnp.int32, (2 * B, PW), 0)
    own_head = (row < B) == (lax.broadcasted_iota(jnp.int32, (2 * B, PW), 1) < DH)
    batch_o = row % B
    batch_s = lax.broadcasted_iota(jnp.int32, (2 * B, W), 0) % B
    first_head = lax.broadcasted_iota(jnp.int32, (B, PW), 1) < DH

    def head_pair(j, acc):
        slot = j % 2
        c = _cols(j, PW)
        q = q_buf[:, c]
        q = jnp.where(own_head, jnp.concatenate([q, q], axis=0), 0.0).astype(jnp.bfloat16)
        _wait(k_buf.at[slot], sem_k)

        def scores(b, s):
            pl.when(j + 1 < NP)(lambda: fetch_cache(k_hbm, k_buf, sem_k, j + 1, b))
            pl.when(j + 1 == NP)(lambda: fetch_w1(b))
            return jnp.where(batch_s == b, _dot(q, k_buf[slot, b]), s)

        s = lax.fori_loop(0, B, scores, jnp.zeros((2 * B, W), jnp.float32)) * DH ** -0.5
        e = jnp.exp(s - jnp.max(s, axis=-1, keepdims=True))
        p = (e / jnp.sum(e, axis=-1, keepdims=True)).astype(jnp.bfloat16)
        _wait(v_buf.at[slot], sem_v)

        def values(b, o):
            pl.when(j + 1 < NP)(lambda: fetch_cache(v_hbm, v_buf, sem_v, j + 1, b))
            pl.when(j + 1 == NP)(lambda: fetch_w2_head(b))
            return jnp.where(batch_o == b, _dot_nt(p, v_buf[slot, b]), o)

        o = lax.fori_loop(0, B, values, jnp.zeros((2 * B, PW), jnp.float32))
        o = jnp.where(first_head, o[:B], o[B:]).astype(jnp.bfloat16)
        return acc + _dot(o, wo_buf[_rows(j, PW), :])

    attn = lax.fori_loop(0, NP, head_pair, jnp.zeros((B, D), jnp.float32))

    fetch_w2_rest()
    x = x + mod_buf[2] * attn
    y = _layernorm(_layernorm(x) * (1.0 + mod_buf[4]) + mod_buf[3]).astype(jnp.bfloat16)
    _wait(w1_buf, sem_k)
    u = _dot(y, w1_buf[...]) + b1_buf[...].astype(jnp.float32).reshape(1, F)
    g = jax.nn.gelu(u, approximate=True).astype(jnp.bfloat16)
    mlp = b2_buf[...].astype(jnp.float32).reshape(1, D)
    for lo, hi, sem in ((0, W2_SPLIT, sem_v), (W2_SPLIT, F, sem_w)):
        _wait(w2_buf.at[pl.ds(lo, hi - lo), :], sem)
        mlp = mlp + _dot(g[:, lo:hi], w2_buf[pl.ds(lo, hi - lo), :])
    o_ref[...] = (x + mod_buf[5] * mlp).astype(o_ref.dtype)


@jax.jit
def pallas_adaLN_cond__sliding_block_cached__mixer_channel_mlp__decode_kernel(
    A_x: jax.Array,
    A_k_cache: jax.Array,
    A_v_cache: jax.Array,
    A_wq: jax.Array,
    A_wo: jax.Array,
    B_x: jax.Array,
    B_w1: jax.Array,
    B_b1: jax.Array,
    B_w2: jax.Array,
    B_b2: jax.Array,
    c: jax.Array,
    w_mod: jax.Array,
):
    del B_x
    assert A_k_cache.shape == A_v_cache.shape == (B, H, SK, DH)
    bf16 = jnp.bfloat16
    out = pl.pallas_call(
        _kernel,
        in_specs=[pl.BlockSpec(memory_space=pl.ANY)] * 11,
        out_specs=pl.BlockSpec(memory_space=pltpu.VMEM),
        out_shape=jax.ShapeDtypeStruct((B, D), A_x.dtype),
        scratch_shapes=[
            pltpu.VMEM((2, B, PW, W), bf16),
            pltpu.VMEM((2, B, PW, W), bf16),
            pltpu.VMEM((2, D // 2, H * DH), bf16),
            pltpu.VMEM((H * DH, D), bf16),
            pltpu.VMEM((D, F), bf16),
            pltpu.VMEM((F, D), bf16),
            pltpu.VMEM((2, D // 2, 6 * D), bf16),
            pltpu.VMEM((B, H * DH), jnp.float32),
            pltpu.VMEM((6, B, D), jnp.float32),
            pltpu.VMEM((B, D), bf16),
            pltpu.VMEM((B, D), bf16),
            pltpu.VMEM((F,), bf16),
            pltpu.VMEM((D,), bf16),
            pltpu.SemaphoreType.DMA((3,)),
        ],
        compiler_params=pltpu.CompilerParams(vmem_limit_bytes=64 * 2**20),
    )(
        A_x.reshape(B, D), c, B_b1, B_b2,
        jnp.swapaxes(A_k_cache, 2, 3).reshape(B, NP, PW, SK),
        jnp.swapaxes(A_v_cache, 2, 3).reshape(B, NP, PW, SK),
        A_wq.reshape(2, D // 2, H * DH), A_wo, B_w1, B_w2,
        w_mod.reshape(2, D // 2, 6 * D),
    )
    return out.reshape(B, 1, D)
```
